```python
import os as _os
_os.environ.setdefault("JAX_PLATFORMS", "cpu")
import jax
import jax.numpy as jnp

def _softmax(x, axis=-1):
    return jax.nn.softmax(x, axis=axis)
def _gelu(x):
    return jax.nn.gelu(x, approximate=True)
def _silu(x):
    return jax.nn.silu(x)
def _sigmoid(x):
    return jax.nn.sigmoid(x)
def _layernorm(x, axis=-1, eps=1e-5):
    m = jnp.mean(x, axis=axis, keepdims=True)
    v = jnp.var(x, axis=axis, keepdims=True)
    return (x - m) / jnp.sqrt(v + eps)
def _scatter_add(tgt, idx, src, axis=0):
    return tgt.at[idx].add(src)
def _segment_sum(src, seg, n):
    return jax.ops.segment_sum(src, seg, n)
class _Rng:
    def __init__(self, key):
        self._k = key
    def _next(self):
        self._k, sub = jax.random.split(self._k)
        return sub
    def normal(self, shape):
        return jax.random.normal(self._next(), shape, dtype=jnp.bfloat16)
    def randint(self, lo, hi, shape):
        return jax.random.randint(self._next(), shape, lo, hi, dtype=jnp.int32)
    def uniform(self, shape, lo=0.0, hi=1.0):
        return jax.random.uniform(self._next(), shape, jnp.bfloat16, lo, hi)
    def permutation(self, n):
        return jax.random.permutation(self._next(), n)


kernel_name = 'gated_mix__ssm_conv_s5__glu_gated_geglu__prompt'

def setup_inputs():
    _rng = _Rng(jax.random.key(int.from_bytes(__import__("os").urandom(4), "little")))
    _w = (lambda a: (lambda t: t.astype(jnp.bfloat16) if jnp.issubdtype(t.dtype, jnp.floating) else t)(jnp.asarray(a)))
    def _A_setup():
        B, S, D = 1, 2048, 448
        P = D
        Lambda_re = -0.5 * jnp.exp((lambda *s: _rng.normal(s) * 0.4)(P))
        Lambda_im = (lambda *s: _rng.normal(s) * 0.4)(P) * 1.0
        B_re = (lambda *s: _rng.normal(s) * 0.4)(P, D) * (D ** -0.5)
        B_im = (lambda *s: _rng.normal(s) * 0.4)(P, D) * (D ** -0.5)
        C_re = (lambda *s: _rng.normal(s) * 0.4)(D, P) * (P ** -0.5)
        C_im = (lambda *s: _rng.normal(s) * 0.4)(D, P) * (P ** -0.5)
        log_dt = (lambda *s: _rng.normal(s) * 0.4)(P) * 0.3 - 2.0
        Dskip = (lambda *s: _rng.normal(s) * 0.4)(D)
        return {
            "x": _w((lambda *s: _rng.normal(s) * 0.05)(B, S, D)),
            "Lambda_re": _w(Lambda_re),
            "Lambda_im": _w(Lambda_im),
            "B_re": _w(B_re),
            "B_im": _w(B_im),
            "C_re": _w(C_re),
            "C_im": _w(C_im),
            "log_dt": _w(log_dt),
            "Dskip": _w(Dskip),
        }
    _A_in = _A_setup()

    def _B_setup():
        B, S, Dm, Df = 1, 2048, 448, 1792
        return {
            "x": _w((lambda *s: _rng.normal(s) * 0.05)(B, S, Dm)),
            "w_gate": _w((lambda *s: _rng.normal(s) * 1.6)(Dm, Df) * (Dm ** -0.5)),
            "w_up": _w((lambda *s: _rng.normal(s) * 1.6)(Dm, Df) * (Dm ** -0.5)),
            "w_down": _w((lambda *s: _rng.normal(s) * 1.6)(Df, Dm) * (Df ** -0.5)),
        }
    _B_in = _B_setup()

    return {
        "A_x": _A_in["x"],
        "A_Lambda_re": _A_in["Lambda_re"],
        "A_Lambda_im": _A_in["Lambda_im"],
        "A_B_re": _A_in["B_re"],
        "A_B_im": _A_in["B_im"],
        "A_C_re": _A_in["C_re"],
        "A_C_im": _A_in["C_im"],
        "A_log_dt": _A_in["log_dt"],
        "A_Dskip": _A_in["Dskip"],
        "B_x": _B_in["x"],
        "B_w_gate": _B_in["w_gate"],
        "B_w_up": _B_in["w_up"],
        "B_w_down": _B_in["w_down"],
        "gate_w": _w((lambda *s: _rng.normal(s) * 0.05)(448) * 16.0),
    }

def reference(A_x, A_Lambda_re, A_Lambda_im, A_B_re, A_B_im, A_C_re, A_C_im, A_log_dt, A_Dskip, B_x, B_w_gate, B_w_up, B_w_down, gate_w):
    def _A_ref(x, Lambda_re, Lambda_im, B_re, B_im, C_re, C_im, log_dt, Dskip):
        Bsz, L, H = x.shape
        Lam = Lambda_re + 1j * Lambda_im
        Bmat = B_re + 1j * B_im
        Cmat = C_re + 1j * C_im
        dt = jnp.exp(log_dt)
        Lam_bar = jnp.exp(dt * Lam)
        B_bar = ((Lam_bar - 1.0) / Lam)[:, None] * Bmat
        Bu = jnp.einsum("bld,pd->blp", x + 0j, B_bar)
        h = jnp.zeros_like(Bu[:, 0, :])
        hs = []
        for t in range(L):
            h = Lam_bar[None, :] * h + Bu[:, t, :]
            hs.append(h)
        hseq = jnp.stack(hs, 1)
        y = 2.0 * jnp.einsum("blp,dp->bld", hseq, Cmat).real + x * Dskip[None, None, :]
        return y

    def _B_ref(x, w_gate, w_up, w_down):
        g = jnp.einsum("bsd,df->bsf", x, w_gate)
        u = jnp.einsum("bsd,df->bsf", x, w_up)
        h = _gelu(g) * u
        return jnp.einsum("bsf,fd->bsd", h, w_down)

    x = A_x
    g = _sigmoid((x * gate_w).sum(-1, keepdims=True))
    a = _A_ref(x, A_Lambda_re, A_Lambda_im, A_B_re, A_B_im, A_C_re, A_C_im, A_log_dt, A_Dskip)
    b = _B_ref(x, B_w_gate, B_w_up, B_w_down)
    return g * a + (1 - g) * b
```

```python
import jax
import jax.numpy as jnp
from jax import lax
import jax.experimental.pallas as pl
import jax.experimental.pallas.tpu as pltpu

_F32 = jnp.float32
_BF16 = jnp.bfloat16

_NT = (((1,), (1,)), ((), ()))
_GELU_C = 0.7978845608028654

_T = 256
_NCH = 8


def _segments(p):
    full = (p // 128) * 128
    segs = [(lo, lo + 128) for lo in range(0, full, 128)]
    if full < p:
        segs.append((full, p))
    return segs


def _hl(a, b):
    parts = []
    for lo, hi in _segments(a.shape[1]):
        parts += [a[:, lo:hi], b[:, lo:hi]]
    return jnp.concatenate(parts, axis=1)


def _lane_tile(col, n):
    return jnp.concatenate([col] * (n // 128), axis=1)


def _kernel(xt_ref, lre_ref, lim_ref, bre_ref, bim_ref, cre_ref, cim_ref,
            ldt_ref, dsk_ref, gw_ref, wg_hbm, wu_hbm, wd_hbm, o_ref,
            wt_s, ct_s, mul_s, carry_s, bu_s, h_s, at_s, col_s,
            wg_s, wu_s, wgut_s, wd_s, sems):
    step = pl.program_id(0)
    d = xt_ref.shape[1]
    seq = xt_ref.shape[2]
    p = lre_ref.shape[0]
    f = wg_s.shape[1]
    q = 2 * p
    nblk = seq // _T
    lc = _T // _NCH
    nreal = q // 128
    ntile = nreal + 1

    def wcopy(i):
        src, dst = ((wg_hbm, wg_s), (wu_hbm, wu_s), (wd_hbm, wd_s))[i]
        return pltpu.make_async_copy(src, dst, sems.at[i])

    @pl.when(step == 0)
    def _phase_a():
        for i in range(3):
            wcopy(i).start()

        lr = lre_ref[...].astype(_F32).reshape(1, p)
        li = lim_ref[...].astype(_F32).reshape(1, p)
        dt = jnp.exp(ldt_ref[...].astype(_F32)).astype(_BF16).astype(_F32).reshape(1, p)
        ea = jnp.exp(dt * lr)
        th = dt * li
        ar = ea * jnp.cos(th)
        ai = ea * jnp.sin(th)
        nr = ar - 1.0
        den = lr * lr + li * li
        cr = (nr * lr + ai * li) / den
        ci = (ai * lr - nr * li) / den

        def sq(r, i):
            return r * r - i * i, 2.0 * (r * i)

        pr, pi = ar, ai
        n = 1
        while n < lc:
            pr, pi = sq(pr, pi)
            n *= 2
        assert n == lc
        rows = [(ar, ai), (pr, pi)]
        for _ in range(2):
            pr, pi = sq(pr, pi)
            rows.append((pr, pi))
        for k, (r, i) in enumerate(rows):
            m1 = jnp.broadcast_to(_hl(r, r), (_NCH, q))
            m2 = jnp.broadcast_to(_hl(-i, i), (_NCH, q))
            for j in range(nreal):
                mul_s[2 * k, j] = m1[:, 128 * j:128 * (j + 1)]
                mul_s[2 * k + 1, j] = m2[:, 128 * j:128 * (j + 1)]
            mul_s[2 * k, nreal] = m1[:, q - 128:q]
            mul_s[2 * k + 1, nreal] = -m2[:, q - 128:q]

        off = 0
        for lo, hi in _segments(p):
            w = hi - lo
            wt_s[off:off + w, :] = bre_ref[lo:hi, :]
            wt_s[off + w:off + 2 * w, :] = bim_ref[lo:hi, :]
            off += 2 * w

        c_re = cre_ref[...].astype(_F32)
        c_im = cim_ref[...].astype(_F32)
        kr = c_re * cr - c_im * ci
        ki = c_re * ci + c_im * cr
        ct_s[...] = _hl(2.0 * kr, -2.0 * ki).astype(_BF16)

        for j, ref in enumerate((dsk_ref, gw_ref)):
            row = ref[...].astype(_F32).reshape(1, d)
            col_s[j] = jnp.broadcast_to(row, (128, d)).T

        for k in range(ntile):
            carry_s[k] = jnp.zeros((_NCH, 128), _F32)

        def mul_tiles(idx):
            return ([mul_s[2 * idx, k] for k in range(ntile)],
                    [mul_s[2 * idx + 1, k] for k in range(ntile)])

        def cmul8(m, st):
            m1, m2 = m
            return [m1[k] * st[k] + m2[k] * st[k ^ 1] for k in range(ntile)]

        sub = lax.broadcasted_iota(jnp.int32, (_NCH, 128), 0)

        def front(i):
            xb = xt_ref[0, :, i * _T:(i + 1) * _T].T
            bu = lax.dot_general(xb, wt_s[...], _NT, preferred_element_type=_F32)
            for k in range(nreal):
                bu_s[i % 2, k] = bu[:, 128 * k:128 * (k + 1)]
            bu_s[i % 2, nreal] = pltpu.roll(bu[:, q - 128:q], 64, 1)

        def scan(i):
            am = mul_tiles(0)
            b = i % 2

            def scan_pass(st, store):
                for t in range(lc + _NCH - 1):
                    rows = pl.ds(t, _NCH, stride=lc - 1)
                    new = [v + bu_s[b, k, rows, :] for k, v in enumerate(cmul8(am, st))]
                    if t < _NCH - 1 or t >= lc:
                        act = jnp.logical_and(sub <= t, sub > t - lc)
                        new = [jnp.where(act, nv, ov) for nv, ov in zip(new, st)]
                    st = new
                    if store:
                        for k in range(nreal):
                            if t >= lc:
                                h_s[b, k, rows, :] = jnp.where(act, st[k], h_s[b, k, rows, :])
                            else:
                                h_s[b, k, rows, :] = st[k]
                return st

            loc = scan_pass([jnp.zeros((_NCH, 128), _F32)] * ntile, store=False)
            v = [pltpu.roll(jnp.where(sub == _NCH - 1, carry_s[k], loc[k]), 1, 0)
                 for k in range(ntile)]
            dd = 1
            idx = 1
            while dd < _NCH:
                sh = [pltpu.roll(vk, dd, 0) for vk in v]
                v = [vk + jnp.where(sub >= dd, ck, 0.0)
                     for vk, ck in zip(v, cmul8(mul_tiles(idx), sh))]
                dd *= 2
                idx += 1
            fin = cmul8(mul_tiles(1), v)
            for k in range(ntile):
                carry_s[k] = loc[k] + fin[k]
            scan_pass(v, store=True)

        def back(i):
            hb = jnp.concatenate([h_s[i % 2, k].astype(_BF16) for k in range(nreal)], axis=1)
            yt = jnp.dot(ct_s[...], hb.T, preferred_element_type=_F32)
            xf = xt_ref[0, :, i * _T:(i + 1) * _T].astype(_F32)
            at_s[:, i * _T:(i + 1) * _T] = yt + xf * _lane_tile(col_s[0], _T)

        pieces = [(w, c) for w in range(2) for c in range(0, f, d)]

        def wpiece(w, c):
            src = (wg_s, wu_s)[w]
            wgut_s[w * f + c:w * f + c + d, :] = src[:, c:c + d].T

        first_piece_stage = 3
        per_stage = 2
        for s in range(nblk + 2):
            if s == first_piece_stage:
                wcopy(0).wait()
                wcopy(1).wait()
            if s < nblk:
                front(s)
            if s >= 2:
                back(s - 2)
            if 1 <= s <= nblk:
                scan(s - 1)
            if s >= first_piece_stage:
                lo = (s - first_piece_stage) * per_stage
                for w, c in pieces[lo:lo + per_stage]:
                    wpiece(w, c)
        assert (nblk + 2 - first_piece_stage) * per_stage >= len(pieces)
        wcopy(2).wait()

    tok = pl.ds(pl.multiple_of(step * _T, 128), _T)
    xt = xt_ref[0, :, tok]
    gu = jnp.dot(wgut_s[...], xt, preferred_element_type=_F32)
    g = gu[:f]
    u = gu[f:]
    inner = g * (_GELU_C + (_GELU_C * 0.044715) * (g * g))
    hg = (0.5 * g) * (1.0 + jnp.tanh(inner)) * u
    bt = jnp.dot(wd_s[...], hg.astype(_BF16), preferred_element_type=_F32)
    xf = xt.astype(_F32)
    gate = jax.nn.sigmoid(jnp.sum(xf * _lane_tile(col_s[1], _T), axis=0, keepdims=True))
    o_ref[0] = gate * at_s[:, tok] + (1.0 - gate) * bt


@jax.jit
def pallas_gated_mix__ssm_conv_s5__glu_gated_geglu__prompt_kernel(
    A_x: jax.Array,
    A_Lambda_re: jax.Array,
    A_Lambda_im: jax.Array,
    A_B_re: jax.Array,
    A_B_im: jax.Array,
    A_C_re: jax.Array,
    A_C_im: jax.Array,
    A_log_dt: jax.Array,
    A_Dskip: jax.Array,
    B_x: jax.Array,
    B_w_gate: jax.Array,
    B_w_up: jax.Array,
    B_w_down: jax.Array,
    gate_w: jax.Array,
):
    del B_x
    bsz, seq, d = A_x.shape
    p = A_Lambda_re.shape[0]
    f = B_w_gate.shape[1]
    q = 2 * p
    assert bsz == 1 and seq % _T == 0 and (_T // _NCH) & (_T // _NCH - 1) == 0
    assert f % d == 0

    def full(shape):
        return pl.BlockSpec(shape, lambda i: (0,) * len(shape))

    hbm = pl.BlockSpec(memory_space=pl.ANY)
    in_specs = [
        full((1, d, seq)),
        full((p,)), full((p,)),
        full((p, d)), full((p, d)),
        full((d, p)), full((d, p)),
        full((p,)), full((d,)), full((d,)),
        hbm, hbm, hbm,
    ]
    x_t = jnp.transpose(A_x, (0, 2, 1))
    wd_t = jnp.transpose(B_w_down, (1, 0))
    out_t = pl.pallas_call(
        _kernel,
        grid=(seq // _T,),
        in_specs=in_specs,
        out_specs=pl.BlockSpec((1, d, _T), lambda i: (0, 0, i)),
        out_shape=jax.ShapeDtypeStruct((bsz, d, seq), _F32),
        scratch_shapes=[
            pltpu.VMEM((q, d), _BF16),
            pltpu.VMEM((d, q), _BF16),
            pltpu.VMEM((8, q // 128 + 1, _NCH, 128), _F32),
            pltpu.VMEM((q // 128 + 1, _NCH, 128), _F32),
            pltpu.VMEM((2, q // 128 + 1, _T, 128), _F32),
            pltpu.VMEM((2, q // 128, _T, 128), _F32),
            pltpu.VMEM((d, seq), _F32),
            pltpu.VMEM((2, d, 128), _F32),
            pltpu.VMEM((d, f), _BF16),
            pltpu.VMEM((d, f), _BF16),
            pltpu.VMEM((2 * f, d), _BF16),
            pltpu.VMEM((d, f), _BF16),
            pltpu.SemaphoreType.DMA((3,)),
        ],
        compiler_params=pltpu.CompilerParams(
            dimension_semantics=("arbitrary",),
            vmem_limit_bytes=100 * 1024 * 1024,
        ),
    )(x_t, A_Lambda_re, A_Lambda_im, A_B_re, A_B_im, A_C_re, A_C_im,
      A_log_dt, A_Dskip, gate_w, B_w_gate, B_w_up, wd_t)
    return jnp.transpose(out_t, (0, 2, 1))
```

```python
import jax
import jax.numpy as jnp
from jax import lax
import jax.experimental.pallas as pl
import jax.experimental.pallas.tpu as pltpu

_F32 = jnp.float32
_BF16 = jnp.bfloat16

_NT = (((1,), (1,)), ((), ()))
_GELU_C = 0.7978845608028654

_T = 256
_NCH = 8
_EARLY = 2
_LAG = 3
_HBUF = _LAG
_PRE = 2


def _segments(p):
    full = (p // 128) * 128
    segs = [(lo, lo + 128) for lo in range(0, full, 128)]
    if full < p:
        segs.append((full, p))
    return segs


def _hl(a, b):
    parts = []
    for lo, hi in _segments(a.shape[1]):
        parts += [a[:, lo:hi], b[:, lo:hi]]
    return jnp.concatenate(parts, axis=1)


def _lane_tile(col, n):
    return jnp.concatenate([col] * (n // 128), axis=1)


def _copy_plan(p, seq):
    names = ["vec0", "vec1", "vec2"]
    for j in range(len(_segments(p))):
        names += ["bre%d" % j, "bim%d" % j]
    names += ["x%d" % i for i in range(_EARLY)] + ["xr"]
    names += ["cre", "cim", "vec3", "vec4", "wg", "wu", "wd"]
    return names


def _kernel(xt_hbm, lre_hbm, lim_hbm, bre_hbm, bim_hbm, cre_hbm, cim_hbm,
            ldt_hbm, dsk_hbm, gw_hbm, wg_hbm, wu_hbm, wd_hbm, o_ref,
            xt_s, v0_s, v1_s, v2_s, v3_s, v4_s, wt_s, cre_s, cim_s, ct_s, mul_s,
            coef_s, carry_s, bu_s, h_s, at_s, col_s, wg_s, wu_s, wgut_s, wd_s, sems):
    step = pl.program_id(0)
    vec_s = (v0_s, v1_s, v2_s, v3_s, v4_s)
    d, seq = xt_s.shape
    p = v0_s.shape[0]
    f = wg_s.shape[1]
    q = 2 * p
    nblk = seq // _T
    lc = _T // _NCH
    nreal = q // 128
    ntile = nreal + 1

    srcdst = {}
    for j, ref in enumerate((lre_hbm, lim_hbm, ldt_hbm, dsk_hbm, gw_hbm)):
        srcdst["vec%d" % j] = (ref, vec_s[j])
    off = 0
    for j, (lo, hi) in enumerate(_segments(p)):
        w = hi - lo
        srcdst["bre%d" % j] = (bre_hbm.at[lo:hi, :], wt_s.at[off:off + w, :])
        srcdst["bim%d" % j] = (bim_hbm.at[lo:hi, :], wt_s.at[off + w:off + 2 * w, :])
        off += 2 * w
    for i in range(_EARLY):
        srcdst["x%d" % i] = (xt_hbm.at[0, :, i * _T:(i + 1) * _T],
                             xt_s.at[:, i * _T:(i + 1) * _T])
    srcdst["xr"] = (xt_hbm.at[0, :, _EARLY * _T:], xt_s.at[:, _EARLY * _T:])
    srcdst["cre"] = (cre_hbm, cre_s)
    srcdst["cim"] = (cim_hbm, cim_s)
    srcdst["wg"] = (wg_hbm, wg_s)
    srcdst["wu"] = (wu_hbm, wu_s)
    srcdst["wd"] = (wd_hbm, wd_s)
    plan = _copy_plan(p, seq)
    assert sorted(plan) == sorted(srcdst)

    def cp(name):
        src, dst = srcdst[name]
        return pltpu.make_async_copy(src, dst, sems.at[plan.index(name)])

    def vrow(j):
        return vec_s[j][...].astype(_F32).reshape(1, p)

    def mul_tiles(idx):
        return ([mul_s[2 * idx, k] for k in range(ntile)],
                [mul_s[2 * idx + 1, k] for k in range(ntile)])

    def cmul8(m, st):
        m1, m2 = m
        return [m1[k] * st[k] + m2[k] * st[k ^ 1] for k in range(ntile)]

    def front(i):
        xb = xt_s[:, i * _T:(i + 1) * _T].T
        bu = lax.dot_general(xb, wt_s[...], _NT, preferred_element_type=_F32)
        for k in range(nreal):
            bu_s[i % 2, k] = bu[:, 128 * k:128 * (k + 1)]
        bu_s[i % 2, nreal] = pltpu.roll(bu[:, q - 128:q], 64, 1)

    def scan(i):
        sub = lax.broadcasted_iota(jnp.int32, (_NCH, 128), 0)
        b = i % 2
        hb_i = i % _HBUF

        def cmul2(idx, pr, st):
            return [mul_s[2 * idx, 2 * pr + j] * st[j] + mul_s[2 * idx + 1, 2 * pr + j] * st[1 - j]
                    for j in range(2)]

        def scan_pass(pr, st, store):
            for t in range(lc + _NCH - 1):
                rows = pl.ds(t, _NCH, stride=lc - 1)
                new = [v + bu_s[b, 2 * pr + j, rows, :] for j, v in enumerate(cmul2(0, pr, st))]
                if t < _NCH - 1 or t >= lc:
                    act = jnp.logical_and(sub <= t, sub > t - lc)
                    new = [jnp.where(act, nv, ov) for nv, ov in zip(new, st)]
                st = new
                if store:
                    for j in range(2):
                        k = 2 * pr + j
                        if k >= nreal:
                            continue
                        if t >= lc:
                            h_s[hb_i, k, rows, :] = jnp.where(act, st[j], h_s[hb_i, k, rows, :])
                        else:
                            h_s[hb_i, k, rows, :] = st[j]
            return st

        prev = None
        for pr in range(ntile // 2):
            zero = jnp.zeros((_NCH, 128), _F32)
            if prev is not None:
                zero = prev * 0.0
            loc = scan_pass(pr, [zero, zero], store=False)
            v = [pltpu.roll(jnp.where(sub == _NCH - 1, carry_s[2 * pr + j], loc[j]), 1, 0)
                 for j in range(2)]
            dd = 1
            idx = 1
            while dd < _NCH:
                sh = [pltpu.roll(vk, dd, 0) for vk in v]
                v = [vk + jnp.where(sub >= dd, ck, 0.0)
                     for vk, ck in zip(v, cmul2(idx, pr, sh))]
                dd *= 2
                idx += 1
            fin = cmul2(1, pr, v)
            for j in range(2):
                carry_s[2 * pr + j] = loc[j] + fin[j]
            prev = scan_pass(pr, v, store=True)[0]

    def back(i):
        hb = jnp.concatenate([h_s[i % _HBUF, k].astype(_BF16) for k in range(nreal)], axis=1)
        yt = jnp.dot(ct_s[...], hb.T, preferred_element_type=_F32)
        xf = xt_s[:, i * _T:(i + 1) * _T].astype(_F32)
        at_s[:, i * _T:(i + 1) * _T] = yt + xf * _lane_tile(col_s[0], _T)

    def stage(s):
        if s < nblk:
            front(s)
        if s >= _LAG:
            back(s - _LAG)
        if 1 <= s <= nblk:
            scan(s - 1)

    @pl.when(step == 0)
    def _s5_head():
        for name in plan:
            cp(name).start()

        for j in range(3):
            cp("vec%d" % j).wait()
        lr = vrow(0)
        li = vrow(1)
        dt = jnp.exp(vrow(2)).astype(_BF16).astype(_F32)
        ea = jnp.exp(dt * lr)
        th = dt * li
        ar = ea * jnp.cos(th)
        ai = ea * jnp.sin(th)
        nr = ar - 1.0
        den = lr * lr + li * li
        coef_s[0:1, :] = (nr * lr + ai * li) / den
        coef_s[1:2, :] = (ai * lr - nr * li) / den

        def sq(r, i):
            return r * r - i * i, 2.0 * (r * i)

        pr, pi = ar, ai
        n = 1
        while n < lc:
            pr, pi = sq(pr, pi)
            n *= 2
        assert n == lc
        rows = [(ar, ai), (pr, pi)]
        for _ in range(2):
            pr, pi = sq(pr, pi)
            rows.append((pr, pi))
        for k, (r, i) in enumerate(rows):
            m1 = jnp.broadcast_to(_hl(r, r), (_NCH, q))
            m2 = jnp.broadcast_to(_hl(-i, i), (_NCH, q))
            for j in range(nreal):
                mul_s[2 * k, j] = m1[:, 128 * j:128 * (j + 1)]
                mul_s[2 * k + 1, j] = m2[:, 128 * j:128 * (j + 1)]
            mul_s[2 * k, nreal] = m1[:, q - 128:q]
            mul_s[2 * k + 1, nreal] = -m2[:, q - 128:q]
        for k in range(ntile):
            carry_s[k] = jnp.zeros((_NCH, 128), _F32)

        for j in range(len(_segments(p))):
            cp("bre%d" % j).wait()
            cp("bim%d" % j).wait()
        for i in range(_EARLY):
            cp("x%d" % i).wait()
        for s in range(_EARLY):
            stage(s)

    @pl.when(step == 1)
    def _s5_rest():
        for name in ("xr", "cre", "cim", "vec3", "vec4"):
            cp(name).wait()

        def prep_out_proj():
            cr2 = 2.0 * coef_s[0:1, :]
            ci2 = 2.0 * coef_s[1:2, :]
            rb = 64
            for r0 in range(0, d, rb):
                c_re = cre_s[r0:r0 + rb, :].astype(_F32)
                c_im = cim_s[r0:r0 + rb, :].astype(_F32)
                ct_s[r0:r0 + rb, :] = _hl(c_re * cr2 - c_im * ci2,
                                          -(c_re * ci2 + c_im * cr2)).astype(_BF16)
            for j in range(2):
                row = vec_s[3 + j][...].astype(_F32).reshape(1, d)
                col_s[j] = jnp.broadcast_to(row, (128, d)).T

        pieces = [(w, c) for w in range(2) for c in range(0, f, d)]
        first_piece_stage = 5
        per_stage = 2
        assert (nblk + _LAG - first_piece_stage) * per_stage >= len(pieces)
        for s in range(_EARLY, nblk + _LAG):
            if s == first_piece_stage:
                cp("wg").wait()
                cp("wu").wait()
            if s == _EARLY:
                front(s)
                prep_out_proj()
                if s >= _LAG:
                    back(s - _LAG)
                scan(s - 1)
            else:
                stage(s)
            if s >= first_piece_stage:
                lo = (s - first_piece_stage) * per_stage
                for w, c in pieces[lo:lo + per_stage]:
                    wgut_s[w * f + c:w * f + c + d, :] = (wg_s, wu_s)[w][:, c:c + d].T
        cp("wd").wait()

    @pl.when(step >= _PRE)
    def _geglu():
        tok = pl.ds(pl.multiple_of((step - _PRE) * _T, 128), _T)
        xt = xt_s[:, tok]
        gu = jnp.dot(wgut_s[...], xt, preferred_element_type=_F32)
        g = gu[:f]
        u = gu[f:]
        inner = g * (_GELU_C + (_GELU_C * 0.044715) * (g * g))
        hg = (0.5 * g) * (1.0 + jnp.tanh(inner)) * u
        bt = jnp.dot(wd_s[...], hg.astype(_BF16), preferred_element_type=_F32)
        xf = xt.astype(_F32)
        gate = jax.nn.sigmoid(
            jnp.sum(xf * _lane_tile(col_s[1], _T), axis=0, keepdims=True))
        o_ref[0] = gate * at_s[:, tok] + (1.0 - gate) * bt


@jax.jit
def pallas_gated_mix__ssm_conv_s5__glu_gated_geglu__prompt_kernel(
    A_x: jax.Array,
    A_Lambda_re: jax.Array,
    A_Lambda_im: jax.Array,
    A_B_re: jax.Array,
    A_B_im: jax.Array,
    A_C_re: jax.Array,
    A_C_im: jax.Array,
    A_log_dt: jax.Array,
    A_Dskip: jax.Array,
    B_x: jax.Array,
    B_w_gate: jax.Array,
    B_w_up: jax.Array,
    B_w_down: jax.Array,
    gate_w: jax.Array,
):
    del B_x
    bsz, seq, d = A_x.shape
    p = A_Lambda_re.shape[0]
    f = B_w_gate.shape[1]
    q = 2 * p
    assert bsz == 1 and seq % _T == 0 and (_T // _NCH) & (_T // _NCH - 1) == 0
    assert f % d == 0 and seq // _T > _EARLY

    x_t = jnp.transpose(A_x, (0, 2, 1))
    wd_t = jnp.transpose(B_w_down, (1, 0))
    out_t = pl.pallas_call(
        _kernel,
        grid=(_PRE + seq // _T,),
        in_specs=[pl.BlockSpec(memory_space=pl.ANY)] * 13,
        out_specs=pl.BlockSpec((1, d, _T), lambda i: (0, 0, jnp.maximum(i - _PRE, 0))),
        out_shape=jax.ShapeDtypeStruct((bsz, d, seq), _F32),
        scratch_shapes=[
            pltpu.VMEM((d, seq), _BF16),
            pltpu.VMEM((p,), _BF16), pltpu.VMEM((p,), _BF16), pltpu.VMEM((p,), _BF16),
            pltpu.VMEM((d,), _BF16), pltpu.VMEM((d,), _BF16),
            pltpu.VMEM((q, d), _BF16),
            pltpu.VMEM((d, p), _BF16),
            pltpu.VMEM((d, p), _BF16),
            pltpu.VMEM((d, q), _BF16),
            pltpu.VMEM((8, q // 128 + 1, _NCH, 128), _F32),
            pltpu.VMEM((8, p), _F32),
            pltpu.VMEM((q // 128 + 1, _NCH, 128), _F32),
            pltpu.VMEM((2, q // 128 + 1, _T, 128), _F32),
            pltpu.VMEM((_HBUF, q // 128, _T, 128), _F32),
            pltpu.VMEM((d, seq), _F32),
            pltpu.VMEM((2, d, 128), _F32),
            pltpu.VMEM((d, f), _BF16),
            pltpu.VMEM((d, f), _BF16),
            pltpu.VMEM((2 * f, d), _BF16),
            pltpu.VMEM((d, f), _BF16),
            pltpu.SemaphoreType.DMA((len(_copy_plan(p, seq)),)),
        ],
        compiler_params=pltpu.CompilerParams(
            dimension_semantics=("arbitrary",),
            vmem_limit_bytes=100 * 1024 * 1024,
        ),
    )(x_t, A_Lambda_re, A_Lambda_im, A_B_re, A_B_im, A_C_re, A_C_im,
      A_log_dt, A_Dskip, gate_w, B_w_gate, B_w_up, wd_t)
    return jnp.transpose(out_t, (0, 2, 1))
```
